```python
import os as _os
_os.environ.setdefault("JAX_PLATFORMS", "cpu")
import jax
import jax.numpy as jnp

def _softmax(x, axis=-1):
    return jax.nn.softmax(x, axis=axis)
def _gelu(x):
    return jax.nn.gelu(x, approximate=True)
def _silu(x):
    return jax.nn.silu(x)
def _sigmoid(x):
    return jax.nn.sigmoid(x)
def _layernorm(x, axis=-1, eps=1e-5):
    m = jnp.mean(x, axis=axis, keepdims=True)
    v = jnp.var(x, axis=axis, keepdims=True)
    return (x - m) / jnp.sqrt(v + eps)
def _scatter_add(tgt, idx, src, axis=0):
    return tgt.at[idx].add(src)
def _segment_sum(src, seg, n):
    return jax.ops.segment_sum(src, seg, n)
class _Rng:
    def __init__(self, key):
        self._k = key
    def _next(self):
        self._k, sub = jax.random.split(self._k)
        return sub
    def normal(self, shape):
        return jax.random.normal(self._next(), shape, dtype=jnp.bfloat16)
    def randint(self, lo, hi, shape):
        return jax.random.randint(self._next(), shape, lo, hi, dtype=jnp.int32)
    def uniform(self, shape, lo=0.0, hi=1.0):
        return jax.random.uniform(self._next(), shape, jnp.bfloat16, lo, hi)
    def permutation(self, n):
        return jax.random.permutation(self._next(), n)


kernel_name = 'concat_heads__ssm_conv_s4__sliding_local_dilated__prompt'

def setup_inputs():
    _rng = _Rng(jax.random.key(int.from_bytes(__import__("os").urandom(4), "little")))
    _w = (lambda a: (lambda t: t.astype(jnp.bfloat16) if jnp.issubdtype(t.dtype, jnp.floating) else t)(jnp.asarray(a)))
    def _A_setup():
        B, L, D, N = 1, 2048, 640, 192
        A_re = -jnp.exp((lambda *s: _rng.normal(s) * 0.8)(D, N))
        A_im = jnp.pi * (lambda *s: _rng.normal(s) * 0.8)(D, N)
        B_re = (lambda *s: _rng.normal(s) * 0.8)(D, N)
        B_im = (lambda *s: _rng.normal(s) * 0.8)(D, N)
        C_re = (lambda *s: _rng.normal(s) * 0.8)(D, N)
        C_im = (lambda *s: _rng.normal(s) * 0.8)(D, N)
        log_dt = (lambda *s: _rng.normal(s) * 0.8)(D) * 0.5 - 4.0
        Dskip = (lambda *s: _rng.normal(s) * 0.05)(D)
        return {
            "u": _w((lambda *s: _rng.normal(s) * 0.05)(B, L, D)),
            "A_re": _w(A_re),
            "A_im": _w(A_im),
            "B_re": _w(B_re),
            "B_im": _w(B_im),
            "C_re": _w(C_re),
            "C_im": _w(C_im),
            "log_dt": _w(log_dt),
            "Dskip": _w(Dskip),
        }
    _A_in = _A_setup()

    def _B_setup():
        B, S, D = 1, 2048, 640
        return {
            "x": _w((lambda *s: _rng.normal(s) * 0.2)(B, S, D)),
            "wqkv": _w((lambda *s: _rng.normal(s) * 0.2)(D, 3 * D)),
            "wo": _w((lambda *s: _rng.normal(s) * 0.05)(D, D)),
        }
    _B_in = _B_setup()

    return {
        "A_u": _A_in["u"],
        "A_A_re": _A_in["A_re"],
        "A_A_im": _A_in["A_im"],
        "A_B_re": _A_in["B_re"],
        "A_B_im": _A_in["B_im"],
        "A_C_re": _A_in["C_re"],
        "A_C_im": _A_in["C_im"],
        "A_log_dt": _A_in["log_dt"],
        "A_Dskip": _A_in["Dskip"],
        "B_x": _B_in["x"],
        "B_wqkv": _B_in["wqkv"],
        "B_wo": _B_in["wo"],
    }

def reference(A_u, A_A_re, A_A_im, A_B_re, A_B_im, A_C_re, A_C_im, A_log_dt, A_Dskip, B_x, B_wqkv, B_wo):
    def _A_ref(u, A_re, A_im, B_re, B_im, C_re, C_im, log_dt, Dskip):
        Bsz, L, D = u.shape
        dt = jnp.exp(log_dt)[:, None]
        A = A_re + 1j * A_im
        Bc = B_re + 1j * B_im
        Cc = C_re + 1j * C_im
        logdA = dt * A
        dB = dt * Bc
        l = (lambda x, dt: x.astype(dt))(jnp.arange(L), A_re.dtype)
        P = jnp.exp(logdA[:, :, None] * l[None, None, :])
        K = jnp.einsum("dn,dnl,dn->dl", Cc, P, dB).real
        L2 = 2 * L
        Kp = jnp.pad(K, ((0, 0), (0, L)))
        up = (lambda x, *d: x.transpose(*d))(u, 0, 2, 1)
        up = jnp.pad(up, ((0, 0), (0, 0), (0, L)))
        Kf = (lambda x, axes=(-2,-1): jnp.fft.rfft2(x.astype(jnp.float32), axes=axes))(Kp[:, None, :], axes=(-2, -1))
        Uf = (lambda x, axes=(-2,-1): jnp.fft.rfft2(x.astype(jnp.float32), axes=axes))(up[:, :, None, :], axes=(-2, -1))
        Yf = Uf * Kf[None, :, :, :]
        y = (lambda x, s, axes=(-2,-1): jnp.fft.irfft2(x, s=s, axes=axes).astype(jnp.bfloat16))(Yf, (1, L2), axes=(-2, -1))[:, :, 0, :L]
        y = (lambda x, *d: x.transpose(*d))(y, 0, 2, 1) + u * Dskip[None, None, :]
        return y

    def _B_ref(x, wqkv, wo):
        B, S, D = x.shape
        H = 32; Dh = D // H
        W, dil = 8, 2
        qkv = (lambda x, *d: x.transpose(*d))((x @ wqkv).reshape(B, S, 3, H, Dh), 2, 0, 3, 1, 4)
        q, k, v = qkv[0], qkv[1], qkv[2]
        scale = Dh ** -0.5
        pos = jnp.arange(S)
        off = jnp.arange(W) * dil
        idx = pos[:, None] - off[None, :]
        mask = idx >= 0
        idx_c = jnp.where(mask, idx, 0).reshape(-1)
        kg = k[:, :, idx_c, :].reshape(B, H, S, W, Dh)
        vg = v[:, :, idx_c, :].reshape(B, H, S, W, Dh)
        logits = jnp.einsum("bhsd,bhswd->bhsw", q, kg) * scale
        logits = jnp.where(mask[None, None, :, :], logits, -1e9)
        attn = _softmax(logits, axis=-1)
        o = jnp.einsum("bhsw,bhswd->bhsd", attn, vg)
        return (lambda x, *d: x.transpose(*d))(o, 0, 2, 1, 3).reshape(B, S, D) @ wo

    a = _A_ref(A_u, A_A_re, A_A_im, A_B_re, A_B_im, A_C_re, A_C_im, A_log_dt, A_Dskip)
    b = _B_ref(B_x, B_wqkv, B_wo)
    return jnp.concatenate([a, b], axis=-1)
```

```python
import ml_dtypes
import numpy as np

import jax
import jax.numpy as jnp
import jax.experimental.pallas as pl
import jax.experimental.pallas.tpu as pltpu

F32 = jnp.float32
BF16 = jnp.bfloat16

L = 2048
D = 640
N = 192
H, DH = 32, 20
W, DIL = 8, 2
NG = D // 128
NC = L // 128
RB = 416
HALO = 16

_L1 = (
    ((0, 4), (1, 5), (2, 6), (3, 7)),
    ((256, 512), (258, 516), (260, 768), (262, 772)),
    ((1024, 1536), (1280, 1792)),
)


def _tables():
    m = np.arange(128)[:, None]
    t = np.arange(128)[None, :]
    x = np.exp(-2j * np.pi * (m + 0.25) * t / 128.0)
    fu = np.concatenate([x.real, x.imag], axis=0)
    fi = fu.T / 128.0
    where = {}
    for q, quad in enumerate(_L1):
        for j, pair in enumerate(quad):
            for e, l1 in enumerate(pair):
                for mm in range(16):
                    for hc in range(2):
                        lane = (8 * mm + 6 + hc + e + 2 * j) % 128
                        tile = hc if q == 0 else 2 * q + e
                        where[l1 + 8 * (mm + 16 * hc)] = (tile, lane)
    lr = np.arange(L).astype(np.float32).astype(ml_dtypes.bfloat16).astype(np.int64)
    mats = {}
    last = np.zeros((256,))
    for l in range(L):
        if lr[l] == L:
            last += fu[:, l % 128]
            continue
        tile, lane = where[int(lr[l])]
        mats.setdefault((l // 128, tile), np.zeros((256, 128)))[:, lane] += fu[:, l % 128]
    passes = tuple(sorted(mats))
    fk = np.stack([fu] + [mats[p] for p in passes])
    last = np.broadcast_to(last[:, None], (256, 128))
    return (passes, fk.astype(np.float32).astype(ml_dtypes.bfloat16),
            fi.astype(np.float32).astype(ml_dtypes.bfloat16),
            np.ascontiguousarray(last, dtype=np.float32))


_PASSES, _FK, _FI, _FLAST = _tables()

_BASE = {}
for _name, _n in (("z8", 3), ("z128", 3), ("z136", 3), ("c8", 4), ("w0", 3), ("w1", 3),
                  ("w256", 3), ("w258", 3), ("c1", 4), ("c2", 4), ("c256", 4)):
    _BASE[_name] = (sum(v[1] for v in _BASE.values()), _n)
_NBASE = sum(v[1] for v in _BASE.values())


def _nt(a, b):
    return jax.lax.dot_general(a, b, (((1,), (1,)), ((), ())), preferred_element_type=F32)


def _nn(a, b):
    return jnp.dot(a, b, preferred_element_type=F32)


def _cmul(a, b):
    return a[0] * b[0] - a[1] * b[1], a[0] * b[1] + a[1] * b[0]


def _interleave(*streams):
    streams = [list(s) for s in streams if s]
    total = [float(sum(c for c, _ in s)) for s in streams]
    done = [0.0] * len(streams)
    pos = [0] * len(streams)
    while True:
        live = [i for i in range(len(streams)) if pos[i] < len(streams[i])]
        if not live:
            return
        i = min(live, key=lambda k: ((done[k] + 0.5 * streams[k][pos[k]][0]) / total[k], k))
        cost, fn = streams[i][pos[i]]
        fn()
        done[i] += cost
        pos[i] += 1


def _kernel(u_h, are_h, aim_h, bre_h, bim_h, cre_h, cim_h, ldt_ref, dsk_ref, x_h, wqkv_h, wo_h,
            fk_h, fi_h, fl_h, out_h,
            par, u_v, x_v, wqkv_v, wo_v, fk_v, fi_v, fl_v, rows, wt32, wq_p, wo_p,
            pre, base, klast, mrg, kt, kf, uf, zz, q_s, k_s, v_s, o_s, ya, yb,
            sem_p, sem_u, sem_x, sem_w, sem_a, sem_b):
    par_h = (are_h, aim_h, bre_h, bim_h, cre_h, cim_h)

    def row0(j):
        return pl.multiple_of(jnp.minimum(j * RB, L - RB), 32)

    def cp_par(j, i):
        return pltpu.make_async_copy(par_h[i].at[:, pl.ds(j * 128, 128)], par.at[j, i], sem_p.at[j])

    def cp_u(j):
        return pltpu.make_async_copy(u_h.at[:, pl.ds(j * 128, 128)], u_v.at[j], sem_u.at[j])

    def cp_x(j):
        r = min(j * RB, L - RB)
        return pltpu.make_async_copy(x_h.at[pl.ds(r, RB), :], x_v.at[j], sem_x.at[j])

    cp_w = [pltpu.make_async_copy(s, d, sem_w.at[i]) for i, (s, d) in enumerate(
        ((wqkv_h, wqkv_v), (wo_h, wo_v), (fk_h, fk_v), (fi_h, fi_v), (fl_h, fl_v)))]

    def cp_a(j):
        col = pl.multiple_of(j * 128, 128)
        return pltpu.make_async_copy(ya.at[j], out_h.at[:, pl.ds(col, 128)], sem_a)

    def cp_b(j):
        return pltpu.make_async_copy(yb.at[j], out_h.at[pl.ds(row0(j), RB), pl.ds(D, D)], sem_b)

    cp_w[0].start()
    for i in range(6):
        cp_par(0, i).start()
    cp_x(0).start()
    cp_w[1].start()
    cp_u(0).start()
    for c in cp_w[2:]:
        c.start()
    for j in range(1, NG):
        for i in range(6):
            cp_par(j, i).start()
        cp_x(j).start()
        cp_u(j).start()

    dt_all = jnp.exp(ldt_ref[...].astype(F32).reshape(1, D)).astype(BF16).astype(F32)
    dsk_all = dsk_ref[...].astype(F32).reshape(1, D)
    for j in range(NG):
        rows[j, 0] = jnp.broadcast_to(dt_all[:, j * 128:(j + 1) * 128], (8, 128))
        rows[j, 1] = jnp.broadcast_to(dsk_all[:, j * 128:(j + 1) * 128], (8, 128))
    for t in range(NG):
        k_s[t, pl.ds(RB, HALO), :] = jnp.zeros((HALO, 128), F32)
        v_s[t, pl.ds(RB, HALO), :] = jnp.zeros((HALO, 128), F32)

    cp_w[0].wait()
    for kk in range(NG):
        for nn in range(3 * NG):
            blk = wqkv_v[pl.ds(kk * 128, 128), pl.ds(nn * 128, 128)].astype(F32)
            wt32[kk, pl.ds(nn * 128, 128), :] = blk.T
        for part in range(3):
            for dh in range(DH):
                wq_p[pl.ds(part * D + dh * H, H), pl.ds(kk * 128, 128)] = (
                    wt32[kk, pl.ds(part * D + dh, H, stride=DH), :].astype(BF16))
    cp_w[1].wait()
    for nn in range(NG):
        wt32[nn, pl.ds(0, D), :] = wo_v[:, pl.ds(nn * 128, 128)].astype(F32)
        for dh in range(DH):
            wo_p[pl.ds(dh * H, H), pl.ds(nn * 128, 128)] = (
                wt32[nn, pl.ds(dh, H, stride=DH), :].astype(BF16))
    for c in cp_w[2:]:
        c.wait()

    sub = jax.lax.broadcasted_iota(jnp.int32, (8, 128), 0)
    lane = jax.lax.broadcasted_iota(jnp.int32, (8, 128), 1)

    def step(j, carry):
        for i in range(6):
            pltpu.make_async_copy(par.at[j, i], par.at[j, i], sem_p.at[j]).wait()
        pltpu.make_async_copy(x_v.at[j], x_v.at[j], sem_x.at[j]).wait()
        pltpu.make_async_copy(u_v.at[j], u_v.at[j], sem_u.at[j]).wait()

        hsrc = pl.multiple_of(jnp.where(j == NG - 1, L - RB - (NG - 2) * RB, RB), 16)
        for t in range(NG):
            k_s[t, pl.ds(0, HALO), :] = k_s[t, pl.ds(hsrc, HALO), :]
            v_s[t, pl.ds(0, HALO), :] = v_s[t, pl.ds(hsrc, HALO), :]

        kacc = []

        def base_rows(r):
            dt = jnp.concatenate([rows[j, 0]] * 2, axis=0)
            a_re, a_im, b_re, b_im, c_re, c_im = (
                par[j, i, pl.ds(r, 16), :].astype(F32) for i in range(6))
            rho = jnp.exp(dt * a_re)
            th = dt * a_im
            z = {1: (rho * jnp.cos(th), rho * jnp.sin(th))}
            coef = {}
            p = 1
            while p < L:
                zr, zi = z[p]
                rr, ii, two = zr * zr, zi * zi, zr + zr
                if p in (1, 2, 8, 256):
                    coef[p] = (two, rr + ii)
                z[2 * p] = (rr - ii, two * zi)
                p *= 2
            w0 = _cmul((c_re, c_im), (dt * b_re, dt * b_im))
            w256 = _cmul(w0, z[256])
            z136 = _cmul(z[128], z[8])
            kl = w0[0] * z[L][0] - w0[1] * z[L][1]
            kacc.append(kl[:8] + kl[8:])
            lo, hi = (r, 128 + r) if r < 128 else (128 + r, 192 + r)

            def put(name, val):
                o = _BASE[name][0] * 128
                pre[pl.ds(o + lo, 16), :] = val[0]
                pre[pl.ds(o + hi, 16), :] = val[1]

            def put_coef(name, val):
                o = _BASE[name][0] * 128
                for i in range(2):
                    pre[pl.ds(o + 256 * i + r, 16), :] = val[i]
                    if r >= 128:
                        pre[pl.ds(o + 256 * i + r + 64, 16), :] = val[i]

            put("z8", (z[8][0], -z[8][1]))
            put("z128", (z[128][0], -z[128][1]))
            put("z136", (z136[0], -z136[1]))
            put("w0", w0)
            put("w1", _cmul(w0, z[1]))
            put("w256", w256)
            put("w258", _cmul(w256, z[2]))
            for p, name in ((8, "c8"), (1, "c1"), (2, "c2"), (256, "c256")):
                put_coef(name, coef[p])

        def base_transpose(i):
            base[i] = pre[pl.ds(i * 128, 128), :].T

        def klast_store():
            s = kacc[0]
            for v in kacc[1:]:
                s = s + v
            klast[...] = jnp.broadcast_to(jnp.sum(s, axis=0, keepdims=True), (8, 128))

        def taps(g):
            def ld(name, i, idx=None):
                v = base[_BASE[name][0] + i, pl.ds(8 * g, 8), :]
                return v if idx is None else jnp.take_along_axis(v, idx, axis=0)

            def run(x0, x1, cname, i, count, idx=None):
                c1, c2 = ld(cname, i // 2, idx), ld(cname, 2 + i // 2, idx)
                xs = [x0, x1]
                while len(xs) < count:
                    xs.append(c1 * xs[-1] - c2 * xs[-2])
                return xs

            low = sub < 4
            lhs = [[], []]
            for i in range(3):
                p = dict(enumerate(run(ld("w0", i), ld("w1", i), "c1", i, 8)))
                p.update(zip(range(256, 264, 2), run(ld("w256", i), ld("w258", i), "c2", i, 4)))
                p.update(zip(range(0, 2048, 256), run(p[0], p[256], "c256", i, 8)))
                p.update(zip(range(4, 1024, 256), run(p[4], p[260], "c256", i, 4)))
                col = [[], []]
                for quad in _L1:
                    for s in range(0, len(quad), 2):
                        xa, xb = (pltpu.pack_elementwise([p[a], p[b]], packed_dtype=BF16)
                                  for a, b in quad[s:s + 2])
                        col[0].append(jnp.where(low, xa, pltpu.roll(xb, 4, 0)))
                        col[1].append(jnp.where(low, pltpu.roll(xa, 4, 0), xb))
                for h in range(2):
                    lhs[h].append(pltpu.bitcast(jnp.concatenate(col[h], axis=0), BF16))
            odd = (sub & 1) == 1
            slot = ((lane - 6 - (sub & 1)) & 7) >> 1
            for h in range(2):
                idx = 4 * h + 3 - (sub >> 1)
                rhs = []
                for i in range(3):
                    one = (jnp.ones((8, 128), F32), jnp.zeros((8, 128), F32),
                           jnp.where(lane < 64, 1.0, 0.0).astype(F32))[i]
                    x0 = jnp.where(odd, ld("z128", i, idx), one)
                    x1 = jnp.where(odd, ld("z136", i, idx), ld("z8", i, idx))
                    rhs.append(jnp.concatenate(run(x0, x1, "c8", i, 16, idx), axis=0).astype(BF16))
                res = _nt(jnp.concatenate(lhs[h], axis=1), jnp.concatenate(rhs, axis=1))
                r = 0
                for q, quad in enumerate(_L1):
                    acc = jnp.zeros((8, 128), F32) if len(quad) < 4 else None
                    for s in range(len(quad)):
                        v = pltpu.roll(res[8 * r:8 * r + 8], 2 * s, 1, stride=1, stride_axis=0)
                        acc = v if acc is None else jnp.where(slot == s, v, acc)
                        r += 1
                    mrg[q, pl.ds(16 * g + 8 * h, 8), :] = acc

        def tap_tiles():
            even = (jax.lax.broadcasted_iota(jnp.int32, (128, 128), 1) & 1) == 0
            for q in range(3):
                t0, t1 = (mrg[q, pl.ds(e, 128, stride=2), :] for e in range(2))
                if q == 0:
                    t0, t1 = jnp.where(even, t0, t1), jnp.where(even, t1, t0)
                kt[2 * q] = t0.astype(BF16)
                kt[2 * q + 1] = t1.astype(BF16)

        def k_dft(c):
            acc = None
            for i, (cc, tile) in enumerate(_PASSES):
                if cc == c:
                    v = _nt(fk_v[1 + i], kt[tile])
                    acc = v if acc is None else acc + v
            if c == NC - 1:
                acc = acc + fl_v[...] * jnp.concatenate([klast[...]] * 32, axis=0)
            kf[c] = acc

        def u_dft(c):
            uf[c] = _nn(fk_v[0], u_v[j, pl.ds(c * 128, 128), :])

        def mac(r):
            def conv(a, b):
                out = []
                for c in range(NC):
                    s = a[0] * b[c]
                    for k in range(1, c + 1):
                        s = s + a[k] * b[c - k]
                    out.append(s)
                return out

            def ld(ref, off):
                return [ref[c, pl.ds(off + r, 8), :] for c in range(NC)]

            p1 = conv(ld(kf, 0), ld(uf, 0))
            p2 = conv(ld(kf, 128), ld(uf, 128))
            p3 = conv([a + b for a, b in zip(ld(kf, 0), ld(kf, 128))],
                      [a + b for a, b in zip(ld(uf, 0), ld(uf, 128))])
            prev = None
            for c in range(NC):
                yr, yi = p1[c] - p2[c], p3[c] - (p1[c] + p2[c])
                zz[c, pl.ds(r, 8), :] = yr if prev is None else yr - prev[1]
                zz[c, pl.ds(128 + r, 8), :] = yi if prev is None else yi + prev[0]
                prev = (yr, yi)

        def i_dft(c):
            y = _nn(fi_v[...], zz[c].astype(BF16))
            skip = u_v[j, pl.ds(c * 128, 128), :].astype(F32) * jnp.concatenate([rows[j, 1]] * 16, axis=0)
            ya[j, pl.ds(c * 128, 128), :] = (y + skip).astype(BF16)

        def proj(part, t):
            res = _nt(x_v[j], wq_p[pl.ds(part * D + t * 128, 128), :])
            if part == 0:
                q_s[t] = res
                return
            (k_s, v_s)[part - 1][t, pl.ds(HALO, RB), :] = res
            if part == 2:
                v_s[t, pl.ds(0, HALO), :] = jnp.where(
                    j == 0, jnp.broadcast_to(res[0:1], (HALO, 128)), v_s[t, pl.ds(0, HALO), :])

        scale = DH ** -0.5

        def attend(r, n):
            q = [q_s[t, pl.ds(r, n), :] for t in range(NG)]
            logit = []
            for w in range(W):
                s = None
                for t in range(NG):
                    p = q[t] * k_s[t, pl.ds(HALO + r - DIL * w, n), :]
                    s = p if s is None else s + p
                s = s + pltpu.roll(s, 64, 1)
                s = s + pltpu.roll(s, 32, 1)
                if r < DIL * w:
                    pos = j * RB + r + jax.lax.broadcasted_iota(jnp.int32, (n, 128), 0)
                    s = jnp.where(pos >= DIL * w, s, -1e9 / scale)
                logit.append(s)
            m = logit[0]
            for s in logit[1:]:
                m = jnp.maximum(m, s)
            e = [jnp.exp2((s - m) * (scale * np.log2(np.e))) for s in logit]
            den = e[0]
            for s in e[1:]:
                den = den + s
            inv = 1.0 / den
            for t in range(NG):
                o = None
                for w in range(W):
                    p = e[w] * v_s[t, pl.ds(HALO + r - DIL * w, n), :]
                    o = p if o is None else o + p
                o_s[pl.ds(r, n), pl.ds(t * 128, 128)] = (o * inv).astype(BF16)

        def out_proj(r, n):
            yb[j, pl.ds(r, n), :] = _nn(o_s[pl.ds(r, n), :], wo_p[...]).astype(BF16)

        def tasks(cost, fn, args):
            return [(cost, (lambda a=a: fn(*a))) for a in args]

        gen = (tasks(150, base_rows, [(r,) for r in range(0, N, 16)])
               + tasks(10, klast_store, [()])
               + tasks(40, base_transpose, [(i,) for i in range(_NBASE)])
               + tasks(170, taps, [(g,) for g in range(16)])
               + tasks(50, tap_tiles, [()]))
        _interleave(gen,
                    tasks(1, proj, [(p, t) for p in (1, 2) for t in range(NG)]),
                    tasks(1, u_dft, [(c,) for c in range(NC)]))
        _interleave(tasks(1, k_dft, [(c,) for c in range(NC)]))
        _interleave(tasks(1, mac, [(r,) for r in range(0, 128, 8)]),
                    tasks(1, proj, [(0, t) for t in range(NG)]))
        half = RB // 2
        _interleave(tasks(1, attend, [(r, 16) for r in range(0, half, 16)]),
                    tasks(1, i_dft, [(c,) for c in range(NC)]))
        _interleave(tasks(1, attend, [(r, 16) for r in range(half, RB, 16)]),
                    tasks(1, out_proj, [(0, half)]))
        out_proj(half, half)

        @pl.when(j > 0)
        def _():
            cp_a(j - 1).wait()
            cp_b(j - 1).wait()

        cp_a(j).start()
        cp_b(j).start()
        return carry

    jax.lax.fori_loop(0, NG, step, 0)
    cp_a(NG - 1).wait()
    cp_b(NG - 1).wait()


@jax.jit
def pallas_concat_heads__ssm_conv_s4__sliding_local_dilated__prompt_kernel(
    A_u: jax.Array,
    A_A_re: jax.Array,
    A_A_im: jax.Array,
    A_B_re: jax.Array,
    A_B_im: jax.Array,
    A_C_re: jax.Array,
    A_C_im: jax.Array,
    A_log_dt: jax.Array,
    A_Dskip: jax.Array,
    B_x: jax.Array,
    B_wqkv: jax.Array,
    B_wo: jax.Array,
):
    assert A_u.shape == (1, L, D) and B_x.shape == (1, L, D) and A_A_re.shape == (D, N)
    hbm = pl.BlockSpec(memory_space=pl.ANY)
    vmem = pl.BlockSpec(memory_space=pltpu.VMEM)
    V = pltpu.VMEM
    dma = pltpu.SemaphoreType.DMA
    out = pl.pallas_call(
        _kernel,
        out_shape=jax.ShapeDtypeStruct((L, 2 * D), BF16),
        in_specs=[hbm] * 7 + [vmem] * 2 + [hbm] * 6,
        out_specs=hbm,
        scratch_shapes=[
            V((NG, 6, N, 128), BF16),
            V((NG, L, 128), BF16),
            V((NG, RB, D), BF16),
            V((D, 3 * D), BF16),
            V((D, D), BF16),
            V(_FK.shape, BF16),
            V(_FI.shape, BF16),
            V(_FLAST.shape, F32),
            V((NG, 2, 8, 128), F32),
            V((NG, 3 * D, 128), F32),
            V((3 * D, D), BF16),
            V((D, D), BF16),
            V((_NBASE * 128, 128), F32),
            V((_NBASE, 128, 128), F32),
            V((8, 128), F32),
            V((3, 256, 128), F32),
            V((6, 128, 128), BF16),
            V((NC, 256, 128), F32),
            V((NC, 256, 128), F32),
            V((NC, 256, 128), F32),
            V((NG, RB, 128), F32),
            V((NG, HALO + RB, 128), F32),
            V((NG, HALO + RB, 128), F32),
            V((RB, D), BF16),
            V((NG, L, 128), BF16),
            V((NG, RB, D), BF16),
            dma((NG,)), dma((NG,)), dma((NG,)), dma((5,)), dma(()), dma(()),
        ],
        compiler_params=pltpu.CompilerParams(vmem_limit_bytes=100 * 1024 * 1024),
    )(A_u.reshape(L, D), A_A_re.T, A_A_im.T, A_B_re.T, A_B_im.T, A_C_re.T, A_C_im.T,
      A_log_dt, A_Dskip, B_x.reshape(L, D), B_wqkv, B_wo, _FK, _FI, _FLAST)
    return out.reshape(1, L, 2 * D)
```

```python
import numpy as np

import jax
import jax.numpy as jnp
import jax.experimental.pallas as pl
import jax.experimental.pallas.tpu as pltpu

F32 = jnp.float32
BF16 = jnp.bfloat16
U32 = jnp.uint32

L = 2048
D = 640
N = 192
H, DH = 32, 20
W, DIL = 8, 2
NG = D // 128
NC = L // 128
RB = 416
RA = RB // 2
HALO = 16
NZ = 8

_L1 = (
    ((0, 4), (1, 5), (2, 6), (3, 7)),
    ((256, 512), (258, 516), (260, 768), (262, 772)),
    ((1024, 1536), (1280, 1792)),
)
_EDGE = (512, 1024, 2048)


def _pack_rows(a):
    b = a.astype(np.float32).astype(np.dtype(BF16)).view(np.uint16).astype(np.uint32)
    return np.ascontiguousarray(b[..., 0::2, :] | (b[..., 1::2, :] << 16))


def _tables():
    m = np.arange(128)[:, None]
    t = np.arange(128)[None, :]
    x = np.exp(-2j * np.pi * (m + 0.25) * t / 128.0)
    fu = np.stack([x.real.reshape(16, 8, 128), x.imag.reshape(16, 8, 128)], axis=1)
    fu = fu.reshape(256, 128)
    fi = fu.T / 128.0
    where = {}
    for q, quad in enumerate(_L1):
        for j, pair in enumerate(quad):
            for e, l1 in enumerate(pair):
                for mm in range(16):
                    for hc in range(2):
                        lane = (8 * mm + 4 * hc + 3 + 4 * e + j + (2 * e if q == 2 else 0)) % 128
                        tile = (hc, 2 + e, 4)[q]
                        where[l1 + 8 * (mm + 16 * hc)] = (tile, lane)
    lr = np.arange(L).astype(np.float32).astype(np.dtype(BF16)).astype(np.int64)
    mats = {}
    last = np.zeros((len(_EDGE), 256))
    for l in range(L):
        if lr[l] in _EDGE and lr[l] > l:
            last[_EDGE.index(lr[l])] += fu[:, l % 128]
            continue
        tile, lane = where[int(lr[l])]
        mats.setdefault((l // 128, tile), np.zeros((256, 128)))[:, lane] += fu[:, l % 128]
    passes = tuple(sorted(mats))
    fk = np.stack([fu] + [mats[p] for p in passes])
    assert [c for c, _ in passes] == list(range(NC))
    last = np.broadcast_to(last[:, :, None], last.shape + (128,))
    return passes, _pack_rows(fk), _pack_rows(fi), np.ascontiguousarray(last, dtype=np.float32)


_PASSES, _FK, _FI, _FLAST = _tables()

_BASE = {}
for _name, _n in (("z8", 3), ("z128", 3), ("z136", 3), ("c8", 4), ("w0", 3), ("w1", 3),
                  ("w256", 3), ("w258", 3), ("c1", 4), ("c2", 4), ("c256", 4)):
    _BASE[_name] = (sum(v[1] for v in _BASE.values()), _n)
_NBASE = sum(v[1] for v in _BASE.values())


def _nt(a, b):
    return jax.lax.dot_general(a, b, (((1,), (1,)), ((), ())), preferred_element_type=F32)


def _nn(a, b):
    return jnp.dot(a, b, preferred_element_type=F32)


def _get(ref, lead, row, n):
    words = ref if ref.dtype == U32 else ref.bitcast(U32)
    return pltpu.bitcast(words[(*lead, pl.ds(row // 2, n // 2), slice(None))], BF16)


def _put(ref, lead, row, val):
    ref[(*lead, pl.ds(row, val.shape[0]), slice(None))] = val.astype(BF16)


def _cmul(a, b):
    return a[0] * b[0] - a[1] * b[1], a[0] * b[1] + a[1] * b[0]


def _interleave(*streams):
    def pieces(stream):
        for cost, n, gen in stream:
            for _ in gen():
                yield cost / n

    streams = [s for s in streams if s]
    total = [float(sum(t[0] for t in s)) for s in streams]
    gens = [pieces(s) for s in streams]
    done = [0.0] * len(streams)
    live = list(range(len(streams)))
    while live:
        i = min(live, key=lambda k: (done[k] / total[k], k))
        cost = next(gens[i], None)
        if cost is None:
            live.remove(i)
        else:
            done[i] += cost


def _kernel(u_h, are_h, aim_h, bre_h, bim_h, cre_h, cim_h, ldt_h, dsk_h, x_h, wqkv_h, wo_h,
            fk_h, fi_h, fl_h, out_h,
            par, ldt_v, dsk_v, u_v, x_v, wqkv_v, wo_v, fk_v, fi_v, fl_v, rows, wt32, wq_p, wo_p,
            pw, pz, pre, base, klast, kt32, kt, sp, raw, q_s, k_s, v_s, lg, o_s, ya, yb, zero,
            sem_i, sem_q, sem_w, sem_o):
    par_h = (are_h, aim_h, bre_h, bim_h, cre_h, cim_h)

    def row0(j):
        if isinstance(j, int):
            return min(j * RB, L - RB)
        return pl.multiple_of(jnp.minimum(j * RB, L - RB), 16)

    def col0(j):
        return j * 128 if isinstance(j, int) else pl.multiple_of(j * 128, 128)

    def cp_par(j):
        return [pltpu.make_async_copy(par_h[i].at[:, pl.ds(col0(j), 128)], par.at[i], sem_i.at[0])
                for i in range(6)]

    def cp_u(j):
        return [pltpu.make_async_copy(u_h.at[:, pl.ds(col0(j), 128)], u_v, sem_i.at[1])]

    def cp_x(j, hf):
        return [pltpu.make_async_copy(x_h.at[pl.ds(row0(j) + hf * RA, RA), pl.ds(kk * 128, 128)],
                                      x_v[hf].at[kk], sem_i.at[2 + hf]) for kk in range(NG)]

    def start(copies):
        for c in copies:
            c.start()

    def wait(copies):
        for c in copies:
            c.wait()

    def wait_all(buf, sem):
        pltpu.make_async_copy(buf, buf, sem_i.at[sem]).wait()

    def cp_q(kk):
        ks = pl.ds(kk * 128, 128)
        return pltpu.make_async_copy(wqkv_h.at[ks, :], wqkv_v.at[ks, :], sem_q.at[kk])

    cp_w = [pltpu.make_async_copy(s, d, sem_w.at[i]) for i, (s, d) in enumerate(
        ((ldt_h, ldt_v), (dsk_h, dsk_v), (fk_h, fk_v), (fl_h, fl_v), (fi_h, fi_v))
        + tuple((wo_h.at[:, pl.ds(nn * 128, 128)], wo_v.at[nn]) for nn in range(NG)))]

    def cp_out(j):
        return [pltpu.make_async_copy(ya, out_h.at[:, pl.ds(col0(j), 128)], sem_o.at[0]),
                pltpu.make_async_copy(yb, out_h.at[pl.ds(row0(j), RB), pl.ds(D, D)], sem_o.at[1])]

    def tasks(cost, n, fn, args):
        return [(cost, n, (lambda a=a: fn(*a))) for a in args]

    def base_tasks(j, slot):
        kacc = []

        def base_rows(r):
            dt = rows[j, 0]
            a_re, a_im, b_re, b_im, c_re, c_im = (
                par[i, pl.ds(r // 16 * 16, 16), :].astype(F32)[r % 16:r % 16 + 8] for i in range(6))
            rho = jnp.exp(dt * a_re)
            th = dt * a_im
            z = {1: (rho * jnp.cos(th), rho * jnp.sin(th))}
            yield
            coef = {}
            p = 1
            while p < L:
                zr, zi = z[p]
                rr, ii, two = zr * zr, zi * zi, zr + zr
                if p in (1, 2, 8, 256):
                    coef[p] = (two, rr + ii)
                z[2 * p] = (rr - ii, two * zi)
                p *= 2
                if p in (8, 64, 512, L):
                    yield
            w0 = _cmul((c_re, c_im), (dt * b_re, dt * b_im))
            w256 = _cmul(w0, z[256])
            z136 = _cmul(z[128], z[8])
            kl = [w0[0] * z[e][0] - w0[1] * z[e][1] for e in _EDGE]
            kacc[:] = [a + b for a, b in zip(kacc, kl)] if kacc else kl
            lo, hi = (r, 128 + r) if r < 128 else (128 + r, 192 + r)

            def put(name, val):
                o = _BASE[name][0] * 128
                pre[pl.ds(o + lo, 8), :] = val[0]
                pre[pl.ds(o + hi, 8), :] = val[1]

            def put_coef(name, val):
                o = _BASE[name][0] * 128
                for i in range(2):
                    pre[pl.ds(o + 256 * i + r, 8), :] = val[i]
                    if r >= 128:
                        pre[pl.ds(o + 256 * i + r + 64, 8), :] = val[i]

            put("z8", (z[8][0], -z[8][1]))
            put("z128", (z[128][0], -z[128][1]))
            put("z136", (z136[0], -z136[1]))
            yield
            put("w0", w0)
            put("w1", _cmul(w0, z[1]))
            put("w256", w256)
            put("w258", _cmul(w256, z[2]))
            for p, name in ((8, "c8"), (1, "c1"), (2, "c2"), (256, "c256")):
                put_coef(name, coef[p])
            yield

        def klast_store():
            for i, s in enumerate(kacc):
                klast[slot, i] = jnp.broadcast_to(jnp.sum(s, axis=0, keepdims=True), (8, 128))
            yield

        def base_transpose(i):
            base[i] = pre[pl.ds(i * 128, 128), :].T
            yield

        return (tasks(68, 7, base_rows, [(r,) for r in range(0, N, 8)])
                + tasks(10, 1, klast_store, [()]),
                tasks(40, 1, base_transpose, [(i,) for i in range(_NBASE)]))

    start(cp_par(0))
    cp_w[0].start()
    cp_w[1].start()
    cp_q(0).start()

    cp_w[0].wait()
    cp_w[1].wait()
    cp_q(1).start()
    dt_all = jnp.exp(ldt_v[...].astype(F32).reshape(1, D)).astype(BF16).astype(F32)
    dsk_all = dsk_v[...].astype(F32).reshape(1, D)
    for j in range(NG):
        rows[j, 0] = jnp.broadcast_to(dt_all[:, j * 128:(j + 1) * 128], (8, 128))
        rows[j, 1] = jnp.broadcast_to(dsk_all[:, j * 128:(j + 1) * 128], (8, 128))
    for t in range(NG):
        k_s[t, pl.ds(RB, HALO), :] = jnp.zeros((HALO, 128), F32)
        v_s[t, pl.ds(RB, HALO), :] = jnp.zeros((HALO, 128), F32)

    def fill(i, c):
        zero[i] = i >> 16
        return c

    jax.lax.fori_loop(0, NZ, fill, 0)
    eye = (jax.lax.broadcasted_iota(jnp.int32, (128, 128), 0)
           == jax.lax.broadcasted_iota(jnp.int32, (128, 128), 1)).astype(BF16)

    def relayout(kk, part):
        for nn in range(part * NG, (part + 1) * NG):
            wt32[kk, pl.ds(nn * 128, 128), :] = _nt(
                eye, wqkv_v[pl.ds(kk * 128, 128), pl.ds(nn * 128, 128)])
            yield
        for dh in range(DH):
            _put(wq_p, (kk,), part * D + dh * H, wt32[kk, pl.ds(part * D + dh, H, stride=DH), :])
        yield

    wait_all(par, 0)
    cp_q(2).start()
    first_rows, first_tiles = base_tasks(0, 0)
    _interleave(first_rows[:5])
    for kk, work in enumerate((first_rows[5:13], first_rows[13:21], first_rows[21:] + first_tiles[:9],
                               first_tiles[9:23], first_tiles[23:])):
        cp_q(kk).wait()
        if kk + 3 < NG:
            cp_q(kk + 3).start()
        elif kk + 3 == NG:
            start(cp_x(0, 0))
        elif kk + 2 == NG:
            start(cp_par(1))
        _interleave(work, tasks(1, NG + 1, relayout, [(kk, part) for part in range(3)]))

    sub = jax.lax.broadcasted_iota(jnp.int32, (8, 128), 0)
    lane = jax.lax.broadcasted_iota(jnp.int32, (8, 128), 1)

    def step(j, carry):
        nxt = jnp.minimum(j + 1, NG - 1)

        wait_all(par, 0)
        wait_all(x_v[0], 2)
        start(cp_u(j))
        start(cp_x(j, 1))

        hsrc = pl.multiple_of(jnp.where(j == NG - 1, L - RB - (NG - 2) * RB, RB), 16)
        for t in range(NG):
            k_s[t, pl.ds(0, HALO), :] = k_s[t, pl.ds(hsrc, HALO), :]
            v_s[t, pl.ds(0, HALO), :] = v_s[t, pl.ds(hsrc, HALO), :]

        low = sub < 4
        ready = set()

        def powers(g):
            def ld(name, i, idx=None):
                v = base[_BASE[name][0] + i, pl.ds(8 * g, 8), :]
                return v if idx is None else jnp.take_along_axis(v, idx, axis=0)

            def coefs(cname, idx=None):
                c = [(ld(cname, t, idx), ld(cname, 2 + t, idx)) for t in range(2)]
                return [c[0], c[0], c[1]]

            def advance(c, x0, x1):
                return [c[i][0] * x1[i] - c[i][1] * x0[i] for i in range(3)]

            p = {e: [ld(name, i) for i in range(3)]
                 for e, name in ((0, "w0"), (1, "w1"), (256, "w256"), (258, "w258"))}
            for cname, stride, exps in (
                    ("c1", 1, range(2, 8)), ("c2", 2, (260, 262)),
                    ("c256", 256, (512, 516, 768, 772, 1024, 1280, 1536, 1792))):
                c = coefs(cname)
                for e in exps:
                    p[e] = advance(c, p[e - 2 * stride], p[e - stride])
                q = ("c1", "c2", "c256").index(cname)
                for qq in ((0,), (), (1, 2))[q]:
                    for i in range(3):
                        _put(pw, (g, 0, i), 32 * qq, jnp.concatenate(
                            [jnp.where(low, p[a][i], pltpu.roll(p[b][i], 4, 0)) for a, b in _L1[qq]], axis=0))
                        _put(pw, (g, 1, i), 32 * qq, jnp.concatenate(
                            [jnp.where(low, pltpu.roll(p[a][i], 4, 0), p[b][i]) for a, b in _L1[qq]], axis=0))
                yield
            for h in range(2):
                idx = 4 * h + 3 - (sub & 3)
                one = (jnp.ones((8, 128), F32), jnp.zeros((8, 128), F32),
                       jnp.where(lane < 64, 1.0, 0.0).astype(F32))
                c = coefs("c8", idx)
                x0 = [jnp.where(low, one[i], ld("z128", i, idx)) for i in range(3)]
                x1 = [jnp.where(low, ld("z8", i, idx), ld("z136", i, idx)) for i in range(3)]
                for m in range(0, 16, 2):
                    if m:
                        x0 = advance(c, x0, x1)
                        x1 = advance(c, x1, x0)
                    for i in range(3):
                        _put(pz, (g, h, i), 8 * m, jnp.concatenate([x0[i], x1[i]], axis=0))
                    if m in (4, 10, 14):
                        yield
            ready.add(("powers", g))

        def taps(g):
            assert ("powers", g) in ready
            slot = (lane - 3) & 3
            mrg = []
            for h in range(2):
                res = None
                for i in range(3):
                    v = _nt(_get(pw, (g, h, i), 0, 80), _get(pz, (g, h, i), 0, 128))
                    res = v if res is None else res + v
                    yield
                mrg.append(res)
            out = []
            for res in mrg:
                r = 0
                for quad in _L1:
                    acc = None
                    for s in range(len(quad)):
                        v = pltpu.roll(res[8 * r:8 * r + 8], s, 1, stride=1, stride_axis=0)
                        acc = v if acc is None else jnp.where(slot == s, v, acc)
                        r += 1
                    out.append(acc)
            first = ((lane - 3) & 7) < 4
            for q in range(3):
                t0 = jnp.where(low, out[q], pltpu.roll(out[3 + q], 4, 0))
                t1 = jnp.where(low, pltpu.roll(out[q], 4, 0), out[3 + q])
                if q == 0:
                    t0, t1 = jnp.where(first, t0, t1), jnp.where(first, t1, t0)
                tiles = (t0, t1) if q < 2 else (jnp.where(slot < 2, t0, pltpu.roll(t1, 2, 1)),)
                for i, v in enumerate(tiles):
                    kt32[2 * q + i, pl.ds(8 * g, 8), :] = v
            yield

        def tap_tiles():
            for i in range(5):
                _put(kt, (i,), 0, kt32[i])
            yield

        def k_dft(c, hf):
            acc = _nt(_get(fk_v, (1 + c,), 128 * hf, 128), _get(kt, (_PASSES[c][1],), 0, 128))
            if 128 * (c + 1) in _EDGE:
                i = _EDGE.index(128 * (c + 1))
                acc = acc + fl_v[i, pl.ds(128 * hf, 128), :] * jnp.concatenate([klast[j, i]] * 16, axis=0)
            put_spectrum(c, hf, acc)
            yield

        def u_dft(c, hf):
            put_spectrum(NC + c, hf, _nn(_get(fk_v, (0,), 128 * hf, 128), _get(u_v, (), c * 128, 128)))
            yield

        def put_spectrum(slot, hf, acc):
            for f in range(8):
                re, im = acc[16 * f:16 * f + 8], acc[16 * f + 8:16 * f + 16]
                sp[slot, pl.ds(24 * (8 * hf + f), 24), :] = jnp.concatenate([re, im, re + im], axis=0)

        def mac(f, part):
            a = [sp[c, pl.ds(24 * f + 8 * part, 8), :] for c in range(NC)]
            b = [sp[NC + c, pl.ds(24 * f + 8 * part, 8), :] for c in range(NC)]

            def conv(x, y):
                out = []
                for c in range(len(x)):
                    s = x[0] * y[c]
                    for k in range(1, c + 1):
                        s = s + x[k] * y[c - k]
                    out.append(s)
                    if c in (3, 5, 6, 7):
                        yield
                return out

            dst = pl.ds(24 * f + 8 * part, 8)
            ee = yield from conv(a[0::2], b[0::2])
            oo = yield from conv(a[1::2], b[1::2])
            for m in range(NC // 2):
                raw[2 * m, dst, :] = ee[m] + oo[m - 1] if m else ee[m]
            both = [p + q for p, q in zip(ee, oo)]
            ss = yield from conv([p + q for p, q in zip(a[0::2], a[1::2])],
                                 [p + q for p, q in zip(b[0::2], b[1::2])])
            for m in range(NC // 2):
                raw[2 * m + 1, dst, :] = ss[m] - both[m]

        def i_dft(c):
            def spectrum(cc, f):
                p1, p2, p3 = (raw[cc, pl.ds(24 * f + 8 * i, 8), :] for i in range(3))
                return p1 - p2, p3 - (p1 + p2)

            zs = []
            for f in range(16):
                yr, yi = spectrum(c, f)
                if c:
                    pr, pi = spectrum(c - 1, f)
                    yr, yi = yr - pi, yi + pr
                zs += [yr, yi]
                if f % 8 == 7:
                    yield
            y = _nn(pltpu.bitcast(fi_v[...], BF16), jnp.concatenate(zs, axis=0).astype(BF16))
            skip = _get(u_v, (), c * 128, 128).astype(F32) * jnp.concatenate([rows[j, 1]] * 16, axis=0)
            ya[pl.ds(c * 128, 128), :] = (y + skip).astype(BF16)
            yield

        def proj(tile, r, n):
            res = None
            for kk in range(NG):
                v = _nt(_get(x_v[r // RA], (kk,), r % RA, n), _get(wq_p, (kk,), tile * 128, 128))
                res = v if res is None else res + v
                if kk + 1 < NG:
                    yield
            part, t = divmod(tile, NG)
            if part == 0:
                q_s[t, pl.ds(r, n), :] = res
            else:
                (k_s, v_s)[part - 1][t, pl.ds(HALO + r, n), :] = res
            if part == 2 and r == 0:
                v_s[t, pl.ds(0, HALO), :] = jnp.where(
                    j == 0, jnp.broadcast_to(res[0:1], (HALO, 128)), v_s[t, pl.ds(0, HALO), :])
            yield

        scale = DH ** -0.5

        def logits(r, n):
            q = [q_s[t, pl.ds(r, n), :] for t in range(NG)]
            part = []
            for w in range(W):
                s = None
                for t in range(NG):
                    p = q[t] * k_s[t, pl.ds(HALO + r - DIL * w, n), :]
                    s = p if s is None else s + p
                part.append(s)
                if w % 2:
                    yield
            part = [(s + pltpu.roll(s, 2 * H, 1)) + (pltpu.roll(s, H, 1) + pltpu.roll(s, 3 * H, 1))
                    for s in part]
            for w, s in enumerate(part):
                if r < DIL * w:
                    pos = j * RB + r + jax.lax.broadcasted_iota(jnp.int32, (n, 128), 0)
                    s = jnp.where(pos >= DIL * w, s, -1e9 / scale)
                lg[w, pl.ds(r, n), :] = s
            yield

        def mix(r, n):
            logit = [lg[w, pl.ds(r, n), :] for w in range(W)]
            m = logit[0]
            for s in logit[1:]:
                m = jnp.maximum(m, s)
            e = [jnp.exp2((s - m) * (scale * np.log2(np.e))) for s in logit]
            den = e[0]
            for s in e[1:]:
                den = den + s
            inv = pl.reciprocal(den, approx=True)
            inv = inv * (2.0 - den * inv)
            yield
            for t in range(NG):
                o = None
                for w in range(W):
                    p = e[w] * v_s[t, pl.ds(HALO + r - DIL * w, n), :]
                    o = p if o is None else o + p
                _put(o_s, (t,), r, o * inv)
                yield
            ready.add(("mix", r))

        def attend(r0, r1):
            def two(r):
                yield from logits(r, 8)
                yield from logits(r + 8, 8)

            a = tasks(50, 10, two, [(r,) for r in range(r0, r1, 16)])
            b = tasks(65, 6, mix, [(r, 16) for r in range(r0, r1, 16)])
            out = a[:2]
            for i in range(len(b)):
                out += a[i + 2:i + 3] + [b[i]]
            return out

        def out_proj(tile, r, n):
            assert ("mix", r + n - 16) in ready
            res = None
            for kk in range(NG):
                v = _nn(_get(o_s, (kk,), r, n), _get(wo_p, (tile,), kk * 128, 128))
                res = v if res is None else res + v
                if kk + 1 < NG:
                    yield
            yb[pl.ds(r, n), pl.ds(tile * 128, 128)] = res.astype(BF16)
            yield

        def matmuls(fn, ntiles, blocks):
            return [task for r, n in blocks
                    for task in tasks(n * NG / 4, NG, fn, [(t, r, n) for t in range(ntiles)])]

        def phase(*streams):
            pl.when(zero[0] == 0)(lambda: _interleave(*streams))

        rows_a = ((0, 96), (96, 112))
        rows_b = ((208, 80), (288, 64), (352, 64))
        nxt_rows, nxt_tiles = base_tasks(nxt, j + 1)
        halves = [(c, hf) for c in range(NC) for hf in range(2)]
        idle = tasks(1, 1, lambda: iter((None,)), [()])
        phase(tasks(1, 9, powers, [(g,) for g in range(16)]) + idle * 3,
              idle + tasks(1, 7, taps, [(g,) for g in range(16)]) + tasks(0.2, 1, tap_tiles, [()]) + idle,
              nxt_rows + idle * 100,
              matmuls(proj, 3 * NG, rows_a))
        wait(cp_u(j))
        wait_all(x_v[1], 3)
        start(cp_x(nxt, 0))
        start(cp_par(jnp.minimum(j + 2, NG - 1)))

        @pl.when(j == 0)
        def _():
            wait(cp_w[2:])
            for nn in range(NG):
                for dh in range(0, DH, 2):
                    pair = wo_v.bitcast(U32)[nn, pl.ds(dh // 2, H, stride=DH // 2), :]
                    for i, bits in enumerate((pair << 16, pair & np.uint32(0xFFFF0000))):
                        _put(wo_p, (nn,), (dh + i) * H, pltpu.bitcast(bits, F32))

        pl.when(j > 0)(lambda: wait(cp_out(j - 1)))
        phase(attend(0, RA),
              tasks(1, 1, u_dft, halves) + tasks(1, 1, k_dft, halves))
        phase(tasks(1, 12, mac, [(f, p) for f in range(16) for p in range(3)]),
              nxt_tiles,
              matmuls(proj, 3 * NG, rows_b))
        _interleave(attend(RA, RB) + idle * 500,
                    idle * 3000 + tasks(64, 3, i_dft, [(c,) for c in range(NC)]),
                    matmuls(out_proj, NG, ((0, 208), (208, 112), (320, 96))))
        start(cp_out(j))
        return carry

    start(cp_w[2:])
    jax.lax.fori_loop(0, NG, step, 0)
    wait_all(x_v[0], 2)
    wait_all(par, 0)
    wait(cp_out(NG - 1))


@jax.jit
def pallas_concat_heads__ssm_conv_s4__sliding_local_dilated__prompt_kernel(
    A_u: jax.Array,
    A_A_re: jax.Array,
    A_A_im: jax.Array,
    A_B_re: jax.Array,
    A_B_im: jax.Array,
    A_C_re: jax.Array,
    A_C_im: jax.Array,
    A_log_dt: jax.Array,
    A_Dskip: jax.Array,
    B_x: jax.Array,
    B_wqkv: jax.Array,
    B_wo: jax.Array,
):
    assert A_u.shape == (1, L, D) and B_x.shape == (1, L, D) and A_A_re.shape == (D, N)
    hbm = pl.BlockSpec(memory_space=pl.ANY)
    V = pltpu.VMEM
    dma = pltpu.SemaphoreType.DMA
    out = pl.pallas_call(
        _kernel,
        out_shape=jax.ShapeDtypeStruct((L, 2 * D), BF16),
        in_specs=[hbm] * 15,
        out_specs=hbm,
        scratch_shapes=[
            V((6, N, 128), BF16),
            V((D,), BF16),
            V((D,), BF16),
            V((L, 128), BF16),
            [V((NG, RA, 128), BF16)] * 2,
            V((D, 3 * D), BF16),
            V((NG, D, 128), BF16),
            V(_FK.shape, jnp.uint32),
            V(_FI.shape, jnp.uint32),
            V(_FLAST.shape, F32),
            V((NG, 2, 8, 128), F32),
            V((NG, 3 * D, 128), F32),
            V((NG, 3 * D, 128), BF16),
            V((NG, D, 128), BF16),
            V((16, 2, 3, 80, 128), BF16),
            V((16, 2, 3, 128, 128), BF16),
            V((_NBASE * 128, 128), F32),
            V((_NBASE, 128, 128), F32),
            V((NG + 1, 3, 8, 128), F32),
            V((5, 128, 128), F32),
            V((5, 128, 128), BF16),
            V((3 * NC, 384, 128), F32),
            V((NC, 384, 128), F32),
            V((NG, RB, 128), F32),
            V((NG, HALO + RB, 128), F32),
            V((NG, HALO + RB, 128), F32),
            V((W, RB, 128), F32),
            V((NG, RB, 128), BF16),
            V((L, 128), BF16),
            V((RB, D), BF16),
            pltpu.SMEM((NZ,), jnp.int32),
            dma((4,)), dma((NG,)), dma((5 + NG,)), dma((2,)),
        ],
        compiler_params=pltpu.CompilerParams(vmem_limit_bytes=100 * 1024 * 1024),
    )(A_u.reshape(L, D), A_A_re.T, A_A_im.T, A_B_re.T, A_B_im.T, A_C_re.T, A_C_im.T,
      A_log_dt, A_Dskip, B_x.reshape(L, D), B_wqkv, B_wo, _FK, _FI, _FLAST)
    return out.reshape(1, L, 2 * D)
```
